```python
import os as _os
_os.environ.setdefault("JAX_PLATFORMS", "cpu")
import jax
import jax.numpy as jnp

def _softmax(x, axis=-1):
    return jax.nn.softmax(x, axis=axis)
def _gelu(x):
    return jax.nn.gelu(x, approximate=True)
def _silu(x):
    return jax.nn.silu(x)
def _sigmoid(x):
    return jax.nn.sigmoid(x)
def _layernorm(x, axis=-1, eps=1e-5):
    m = jnp.mean(x, axis=axis, keepdims=True)
    v = jnp.var(x, axis=axis, keepdims=True)
    return (x - m) / jnp.sqrt(v + eps)
def _scatter_add(tgt, idx, src, axis=0):
    return tgt.at[idx].add(src)
def _segment_sum(src, seg, n):
    return jax.ops.segment_sum(src, seg, n)
class _Rng:
    def __init__(self, key):
        self._k = key
    def _next(self):
        self._k, sub = jax.random.split(self._k)
        return sub
    def normal(self, shape):
        return jax.random.normal(self._next(), shape, dtype=jnp.bfloat16)
    def randint(self, lo, hi, shape):
        return jax.random.randint(self._next(), shape, lo, hi, dtype=jnp.int32)
    def uniform(self, shape, lo=0.0, hi=1.0):
        return jax.random.uniform(self._next(), shape, jnp.bfloat16, lo, hi)
    def permutation(self, n):
        return jax.random.permutation(self._next(), n)


kernel_name = 'standalone__fft_conv__vision'

def setup_inputs():
    _rng = _Rng(jax.random.key(int.from_bytes(__import__("os").urandom(4), "little")))
    _w = (lambda a: (lambda t: t.astype(jnp.bfloat16) if jnp.issubdtype(t.dtype, jnp.floating) else t)(jnp.asarray(a)))
    H = W = 224
    C = 96
    K = 3
    return {
        "x": _w((lambda *s: _rng.normal(s) * 0.05)(1, H, W, C)),
        "w": _w((lambda *s: _rng.normal(s) * 0.05)(K, K, C, C)),
    }

def reference(x, w):
    B, H, W, C = x.shape
    K = w.shape[0]
    wp = jnp.pad(w, ((0, H - K), (0, W - K), (0, 0), (0, 0)))
    Xf = (lambda x, axes=(-2,-1): jnp.fft.rfft2(x.astype(jnp.float32), axes=axes))(x, axes=(1, 2))
    Wf = (lambda x, axes=(-2,-1): jnp.fft.rfft2(x.astype(jnp.float32), axes=axes))(wp, axes=(0, 1))
    Yf = jnp.einsum('bhwi,hwio->bhwo', Xf, Wf)
    y = (lambda x, s, axes=(-2,-1): jnp.fft.irfft2(x, s=s, axes=axes).astype(jnp.bfloat16))(Yf, (H, W), axes=(1, 2))
    return y
```

```python
import functools
import jax, jax.numpy as jnp
from jax import lax
from jax.experimental import pallas as pl
from jax.experimental.pallas import tpu as pltpu

H = W = 224; C = 96
TH = 8

def kern(x_ref, xh_ref, w_ref, o_ref, s_ref, g_ref):
    i = pl.program_id(0)
    @pl.when(i == 0)
    def _():
        for th in range(3):
            for tw in range(3):
                wt = w_ref[th, tw].astype(jnp.float32).T.astype(jnp.bfloat16)
                g_ref[(2 - th) * 3 + tw] = wt

    def shifted(row):
        out = []
        for tw in range(3):
            if tw == 0:
                out.append(row)
            else:
                out.append(jnp.concatenate([row[:, W - tw:], row[:, :W - tw]], axis=1))
        return out
    for r in range(2):
        for tw, v in enumerate(shifted(xh_ref[r])):
            s_ref[r * 3 + tw] = v
    for r in range(TH):
        for tw, v in enumerate(shifted(x_ref[r])):
            s_ref[(r + 2) * 3 + tw] = v
    for r in range(TH):
        acc = None
        for k in range(9):
            p = jnp.dot(g_ref[k], s_ref[r * 3 + k], preferred_element_type=jnp.float32)
            acc = p if acc is None else acc + p
        o_ref[r] = acc.astype(o_ref.dtype)

@jax.jit
def pallas_standalone__fft_conv__vision_kernel(x, w):
    xt = jnp.transpose(x, (0, 1, 3, 2)).reshape(H, C, W)
    nb = H // TH
    y = pl.pallas_call(
        kern,
        out_shape=jax.ShapeDtypeStruct((H, C, W), x.dtype),
        grid=(nb,),
        in_specs=[pl.BlockSpec((TH, C, W), lambda i: (i, 0, 0)),
                  pl.BlockSpec((2, C, W), lambda i: ((i * (TH // 2) - 1) % (H // 2), 0, 0)),
                  pl.BlockSpec((3, 3, C, C), lambda i: (0, 0, 0, 0))],
        out_specs=pl.BlockSpec((TH, C, W), lambda i: (i, 0, 0)),
        scratch_shapes=[pltpu.VMEM(((TH + 2) * 3, C, W), jnp.bfloat16), pltpu.VMEM((9, C, C), jnp.bfloat16)],
        compiler_params=pltpu.CompilerParams(dimension_semantics=("arbitrary",), vmem_limit_bytes=64 * 1024 * 1024),
    )(xt, xt, w)
    return jnp.transpose(y.reshape(1, H, C, W), (0, 1, 3, 2))
```

```python
import jax, jax.numpy as jnp
from jax import lax
from jax.experimental import pallas as pl
from jax.experimental.pallas import tpu as pltpu

H = W = 224
C = 96
NS = 4
G = H // NS
NT = 7
CP = C // 2
NQ = G // 4
LA = 2
D1 = 2
HOLD = 5
OFF = 2
DS = 4
ORDER = (4, 5, 6, 0, 1, 2, 3)
NV = CP // 8
RB = 768

PA = 2.0 / 3.0
PB = 1.5
A2, B2 = PA * PA, PB * PB

bf16 = jnp.bfloat16
f32 = jnp.float32
u32 = jnp.uint32


def _unpack(v, i):
    return pltpu.unpack_elementwise(v, index=i, packed_dtype=bf16, unpacked_dtype=f32)


def _pack(lo, hi):
    return pltpu.pack_elementwise([lo, hi], packed_dtype=bf16)


def _bt(d):
    d0, d1, d2, d3, d4, d5 = d
    a2d2 = A2 * d2
    b2d3 = B2 * d3
    ea = d4 - B2 * d2
    eb = d4 - a2d2
    oa = A2 * d3 - d1
    ob = b2d3 - d1
    boa = PB * oa
    aob = PA * ob
    return (ea - a2d2 + d0, ea + boa, ea - boa, eb + aob, eb - aob, d5 - b2d3 - oa)


def kern(x_hbm, w_hbm, o_hbm, xb0, xb1, wb, g05, gm, gr, sb, yb0, yb1, sin, sw, sout, zs, *cbs):
    zs[0] = 0
    zs[1] = 0
    zs[2] = G
    Z = [None, None, None]
    xb0h = xb0.bitcast(bf16)
    xb1h = xb1.bitcast(bf16)
    yb0h = yb0.bitcast(bf16)
    yb1h = yb1.bitcast(bf16)

    def in_copies(g0, n, s):
        return (pltpu.make_async_copy(x_hbm.at[:, pl.ds(g0, n), :, pl.ds(0, 128)], xb0h.at[:, pl.ds(g0, n)], sin.at[s]),
                pltpu.make_async_copy(x_hbm.at[:, pl.ds(g0, n), :, pl.ds(128, 96)], xb1h.at[:, pl.ds(g0, n)], sin.at[s]))

    def out_copies(g0, n):
        return (pltpu.make_async_copy(yb0h.at[:, pl.ds(g0, n)], o_hbm.at[:, pl.ds(g0, n), :, pl.ds(0, 128)], sout.at[0]),
                pltpu.make_async_copy(yb1h.at[:, pl.ds(g0, n)], o_hbm.at[:, pl.ds(g0, n), :, pl.ds(128, 96)], sout.at[0]))

    def out_copy0(q, g0, n):
        return pltpu.make_async_copy(yb0h.at[q, pl.ds(g0, n)], o_hbm.at[q, pl.ds(g0, n), :, pl.ds(0, 128)], sout.at[0])

    def out_copy1(g0, n):
        return pltpu.make_async_copy(yb1h.at[:, pl.ds(g0, n)], o_hbm.at[:, pl.ds(g0, n), :, pl.ds(128, 96)], sout.at[0])

    wcp = pltpu.make_async_copy(w_hbm, wb, sw.at[0])
    wcp.start()
    for cp in in_copies(G - 2, 2, 0):
        cp.start()
    for j in range(NQ - 1):
        for cp in in_copies(4 * j, 4, j):
            cp.start()
    for cp in in_copies(G - 4, 2, NQ - 1):
        cp.start()

    wcp.wait()
    wf = [wb[th].reshape(3 * C, C).astype(f32) for th in range(3)]
    ga, gb, gc = wf[2], wf[1], wf[0]
    ur = jnp.concatenate([ga[256:], gb[256:], gc[256:]], axis=0)
    u0 = jnp.concatenate([ga[:256], ur], axis=0)
    u5 = jnp.concatenate([gc[:256], ur], axis=0)
    ga, gb, gc = ga[:256], gb[:256], gc[:256]
    fa = 1.0 / (2 * A2 * (A2 - B2))
    fb = 1.0 / (2 * B2 * (B2 - A2))
    eva = (ga + A2 * gc) * fa
    oda = gb * (PA * fa)
    evb = (ga + B2 * gc) * fb
    odb = gb * (PB * fb)
    ri = lax.broadcasted_iota(jnp.int32, (C, C), 0)
    ci = lax.broadcasted_iota(jnp.int32, (C, C), 1)
    hi_half = ri >= CP
    r2 = jnp.where(hi_half, ri - CP, ri)
    odd = r2 >= CP // 2
    r3 = jnp.where(odd, r2 - CP // 2, r2)
    ch = 4 * r3 + jnp.where(odd, 1, 0) + jnp.where(hi_half, 2, 0)
    pm = jnp.where(ch == ci, 1.0, 0.0).astype(bf16)

    def permpack(u):
        ut = lax.dot_general(pm, u.astype(bf16), (((1,), (1,)), ((), ())), preferred_element_type=f32)
        return _pack(ut[:CP], ut[CP:])
    g05[0] = permpack(u0)
    gr[...] = permpack(ur)
    gm[0] = permpack(eva + oda)
    gm[1] = permpack(eva - oda)
    gm[2] = permpack(evb + odb)
    gm[3] = permpack(evb - odb)
    g05[1] = permpack(u5)

    lane = lax.broadcasted_iota(jnp.int32, (8, 128), 1)

    def ld_e(q, g, k):
        t0 = xb0[q, g + Z[0], pl.ds(8 * k, 8), :]
        t1 = xb1[q, g, pl.ds(8 * k, 8), :]
        return jnp.concatenate([t1, t0[:, 96:]], axis=1)

    def stage_l1(t, rows, k):
        o = []
        for (sh, g) in rows:
            if t < 4:
                o.append(pltpu.roll(ld_e((t + sh) % 4, g, k), 32, 1))
            else:
                o.append(pltpu.roll(ld_e((3 + sh) % 4, g, k), 96 - 32 * (t - 4), 1))
        return o

    def versions(t, rows, k, l1):
        bases = []
        for (sh, g) in rows:
            if t < 4:
                bases.append(xb0[(t + sh) % 4, g + Z[0], pl.ds(8 * k, 8), :])
            else:
                bases.append(ld_e((t - 4 + sh) % 4, g, k))
        v = []
        for tw in range(3):
            if tw == 0:
                v.append(bases if t < 4 else [jnp.where(lane < 96, b, l) for b, l in zip(bases, l1)])
            else:
                m = (lane >= 128 - tw) if t < 4 else ((lane >= 96 - tw) & (lane < 128 - tw))
                v.append([pltpu.roll(jnp.where(m, l, b), tw, 1) for b, l in zip(bases, l1)])
        return v

    def stage_b(t, k, tw, v):
        k0 = tw * CP + 8 * k
        if len(v) == 4:
            d = [sb[0, t, pl.ds(k0, 8), :], sb[1, t, pl.ds(k0, 8), :]] + v
        else:
            d = v
        sb[0, t, pl.ds(k0, 8), :] = d[4]
        sb[1, t, pl.ds(k0, 8), :] = d[5]
        if k0 < 128:
            lo = _bt([_unpack(x, 0) for x in d])
            hi = _bt([_unpack(x, 1) for x in d])
            for c in range(6):
                cbs[t][Z[0], pl.ds(128 * c + k0, 8), :] = _pack(lo[c], hi[c])
        else:
            for i in range(6):
                cbs[t][Z[0], pl.ds(RB + 16 * i + (k0 - 128), 8), :] = d[i]

    lane48 = lax.broadcasted_iota(jnp.int32, (CP, 128), 1)

    def c_rounds(t, g, pieces):
        def ld(a, n):
            return pltpu.bitcast(cbs[t][Z[1], pl.ds(a, n), :], bf16)

        def dot(gw, v):
            return jnp.dot(pltpu.bitcast(gw, bf16), v, preferred_element_type=f32)

        def store(i, y):
            y = _pack(y[:CP], y[CP:])
            if t < 4:
                yb0[t, g + i] = y
            else:
                yb1[t - 4, g + i] = y[:, :96]
                pieces[i].append(y)
        p0 = dot(g05[0], jnp.concatenate([ld(0, 128), ld(RB, 48)], axis=0))
        p2 = dot(gr[...], ld(RB + 32, 48))
        yield p2[0:8]
        yield p2[64:72]
        ap = dot(gm[0], ld(128, 128))
        am = dot(gm[1], ld(256, 128))
        sa = ap + am
        da = ap - am
        p0 = p0 + sa
        p2 = p2 + A2 * sa
        yield da[32:40]
        bp = dot(gm[2], ld(384, 128))
        bm = dot(gm[3], ld(512, 128))
        sbb = bp + bm
        db = bp - bm
        store(0, p0 + sbb)
        store(2, p2 + B2 * sbb)
        p1 = PA * da + PB * db
        p3 = (PA * A2) * da + (PB * B2) * db
        yield db[0:8]
        yield db[64:72]
        store(3, p3 + dot(g05[1], jnp.concatenate([ld(640, 128), ld(RB + 48, 48)], axis=0)))
        r1 = dot(gr[...], ld(RB + 16, 48))
        store(1, p1 + r1)
        yield r1[32:40]

    def stage_d(g, pieces, i):
        p4, p5, p6 = [pltpu.roll(y, 32 * (q + 1), 1) for q, y in enumerate(pieces[i])]
        yb1[3, g + i] = jnp.where(lane48 < 32, p4, jnp.where(lane48 < 64, p5, p6))[:, :96]

    def run_quad(j, first, last):
        Z[0] = zs[0]
        Z[1] = zs[1]
        Z[2] = zs[2]
        n_end = NT if last else NT + LA
        n_beg = 0 if first else LA

        def rows_of(n):
            g = 4 * (j + n // NT)
            r = [(0, g + i) for i in range(4)]
            if first and n < NT:
                r = [(3, G - 2), (3, G - 1)] + r
            return r
        l1 = {}

        def do_l1(m):
            n, k = divmod(m, NV)
            if n < n_end:
                if first and m == NT * NV:
                    for cp in in_copies(4, 4, 1):
                        cp.wait()
                l1[m] = stage_l1(ORDER[n % NT], rows_of(n), k)

        def ab_chunk(m):
            n, k = divmod(m, NV)
            if n >= n_end:
                return
            t = ORDER[n % NT]
            vs = versions(t, rows_of(n), k, l1.pop(m))
            do_l1(m + D1)
            for tw in range(3):
                stage_b(t, k, tw, vs[tw])

        for m in range(n_beg * NV, n_beg * NV + D1):
            do_l1(m)
        for m in range(n_beg * NV, LA * NV + OFF):
            ab_chunk(m)
        m = LA * NV + OFF
        pieces = [[], [], [], []]
        for n in range(NT):
            t = ORDER[n]
            for r, tick in enumerate(c_rounds(t, 4 * j, pieces)):
                if m < n_end * NV:
                    xb0[0, Z[2], pl.ds(0, 8), :] = pltpu.bitcast(tick, u32)
                    ab_chunk(m)
                m += 1
                if n == DS and r < 4:
                    stage_d(4 * j, pieces, r)
                if last and r == 2 and n >= 4:
                    out_copy0(ORDER[n - 1], 4 * j, 4).start()
                    if n == DS + 1:
                        out_copy1(4 * j, 4).start()

    for cp in in_copies(G - 2, 2, 0):
        cp.wait()
    for cp in in_copies(0, 4, 0):
        cp.wait()
    run_quad(0, True, False)

    def body(j, carry):
        @pl.when(j < NQ - 2)
        def _():
            for cp in in_copies(4 * (j + 1), 4, j + 1):
                cp.wait()

        @pl.when(j == NQ - 2)
        def _():
            for cp in in_copies(G - 4, 2, NQ - 1):
                cp.wait()

        @pl.when(j == HOLD + 1)
        def _():
            for cp in out_copies(0, 4 * (HOLD + 1)):
                cp.start()

        @pl.when(j > HOLD + 1)
        def _():
            for cp in out_copies(4 * (j - 1), 4):
                cp.start()
        run_quad(j, False, False)
        return carry

    lax.fori_loop(1, NQ - 1, body, 0)
    for cp in out_copies(4 * (NQ - 2), 4):
        cp.start()
    run_quad(NQ - 1, False, True)
    out_copy0(3, 4 * (NQ - 1), 4).start()
    for cp in out_copies(0, 4 * (HOLD + 1)):
        cp.wait()
    for j in range(HOLD + 1, NQ - 1):
        for cp in out_copies(4 * j, 4):
            cp.wait()
    out_copy1(4 * (NQ - 1), 4).wait()
    for q in range(4):
        out_copy0(q, 4 * (NQ - 1), 4).wait()


@jax.jit
def pallas_standalone__fft_conv__vision_kernel(x, w):
    xt = jnp.transpose(x, (0, 1, 3, 2)).reshape(NS, G, C, W)
    y = pl.pallas_call(
        kern,
        out_shape=jax.ShapeDtypeStruct((NS, G, C, W), x.dtype),
        in_specs=[pl.BlockSpec(memory_space=pl.ANY), pl.BlockSpec(memory_space=pl.ANY)],
        out_specs=pl.BlockSpec(memory_space=pl.ANY),
        scratch_shapes=[
            pltpu.VMEM((NS, G + 1, CP, 128), u32),
            pltpu.VMEM((NS, G, CP, 96), u32),
            pltpu.VMEM((3, 3, C, C), bf16),
            pltpu.VMEM((2, CP, 352), u32),
            pltpu.VMEM((4, CP, 256), u32),
            pltpu.VMEM((CP, 96), u32),
            pltpu.VMEM((2, NT, 144, 128), u32),
            pltpu.VMEM((NS, G, CP, 128), u32),
            pltpu.VMEM((NS, G, CP, 96), u32),
            pltpu.SemaphoreType.DMA((NQ,)),
            pltpu.SemaphoreType.DMA((1,)),
            pltpu.SemaphoreType.DMA((1,)),
            pltpu.SMEM((3,), jnp.int32),
        ] + [pltpu.VMEM((2, RB + 96, 128), u32)] * NT,
        compiler_params=pltpu.CompilerParams(vmem_limit_bytes=100 * 1024 * 1024),
    )(xt, w)
    return jnp.transpose(y.reshape(1, H, C, W), (0, 1, 3, 2))
```

```python
import jax, jax.numpy as jnp
from jax import lax
from jax.experimental import pallas as pl
from jax.experimental.pallas import tpu as pltpu

H = W = 224
C = 96
NS = 4
G = H // NS
NT = 7
CP = C // 2
NQ = G // 4
LA = 2
D1 = 2
D1F = 4
OFF = 2
DS = 4
HOLD = 5
HS = 0
UQ = 1
NP = 4
NB = (NQ - 2) // UQ
BLOCKS = [(1, 1), (UQ, NB), (1, 1)]
ORDER = (4, 5, 6, 0, 1, 2, 3)
KORD = (4, 0, 1, 5, 2, 3)
NV = CP // 8
RB = 768

PA = 2.0 / 3.0
PB = 1.5
A2, B2 = PA * PA, PB * PB

bf16 = jnp.bfloat16
f32 = jnp.float32
u32 = jnp.uint32


def _unpack(v, i):
    return pltpu.unpack_elementwise(v, index=i, packed_dtype=bf16, unpacked_dtype=f32)


def _pack(lo, hi):
    return pltpu.pack_elementwise([lo, hi], packed_dtype=bf16)


def _bt(d):
    d0, d1, d2, d3, d4, d5 = d
    a2d2 = A2 * d2
    b2d3 = B2 * d3
    ea = d4 - B2 * d2
    eb = d4 - a2d2
    oa = A2 * d3 - d1
    ob = b2d3 - d1
    boa = PB * oa
    aob = PA * ob
    return (ea - a2d2 + d0, ea + boa, ea - boa, eb + aob, eb - aob, d5 - b2d3 - oa)


def kern(x_hbm, w_hbm, o_hbm, xb0, xb1, wb, g05, gm, gr, sb, yb0, yb1, sin, sw, sout, zs, *bufs):
    cbs, tbs = bufs[:NT], bufs[NT:]
    zs[0] = 0
    zs[1] = 0
    zs[2] = G
    Z = [None, None, None]
    xb0h = xb0.bitcast(bf16)
    xb1h = xb1.bitcast(bf16)
    yb0h = yb0.bitcast(bf16)
    yb1h = yb1.bitcast(bf16)

    def in_copies(g0, n, s):
        return (pltpu.make_async_copy(x_hbm.at[:, pl.ds(g0, n), :, pl.ds(0, 128)], xb0h.at[:, pl.ds(g0, n)], sin.at[s]),
                pltpu.make_async_copy(x_hbm.at[:, pl.ds(g0, n), :, pl.ds(128, 96)], xb1h.at[:, pl.ds(g0, n)], sin.at[s]))

    def out_copies(j, held):
        ga, na = (0, 4 * j) if held else (4 * (j - UQ), 4 * UQ)
        gb, nb = (0, 4 * (j - 1)) if held else (4 * (j - UQ - 1), 4 * UQ)
        return (pltpu.make_async_copy(yb0h.at[pl.ds(2, 2), pl.ds(gb, nb)], o_hbm.at[pl.ds(2, 2), pl.ds(gb, nb), :, pl.ds(0, 128)], sout.at[0]),
                pltpu.make_async_copy(yb1h.at[:, pl.ds(ga, na)], o_hbm.at[:, pl.ds(ga, na), :, pl.ds(128, 96)], sout.at[0]),
                pltpu.make_async_copy(yb0h.at[pl.ds(0, 2), pl.ds(ga, na)], o_hbm.at[pl.ds(0, 2), pl.ds(ga, na), :, pl.ds(0, 128)], sout.at[0]))

    def tile_copies(p, g0, n=4):
        if p < 4:
            return (pltpu.make_async_copy(yb0h.at[p, pl.ds(g0, n)], o_hbm.at[p, pl.ds(g0, n), :, pl.ds(0, 128)], sout.at[0]),)
        return (pltpu.make_async_copy(yb1h.at[p - 4, pl.ds(g0, n)], o_hbm.at[p - 4, pl.ds(g0, n), :, pl.ds(128, 96)], sout.at[0]),)

    chunks = []
    j0 = 0
    for (nq, reps) in BLOCKS:
        for _ in range(reps):
            chunks.append((4 * j0, min(4 * nq, G - 2 - 4 * j0)))
            j0 += nq
    assert j0 == NQ

    wcp = pltpu.make_async_copy(w_hbm, wb, sw.at[0])
    wcp.start()
    for cp in in_copies(G - 2, 2, 0):
        cp.start()
    for s, (g0, n) in enumerate(chunks):
        for cp in in_copies(g0, n, s):
            cp.start()

    wcp.wait()
    wf = [wb[th].reshape(3 * C, C).astype(f32) for th in range(3)]
    ga, gb, gc = wf[2], wf[1], wf[0]
    ur = jnp.concatenate([ga[256:], gb[256:], gc[256:]], axis=0)
    u0 = jnp.concatenate([ga[:256], ur], axis=0)
    u5 = jnp.concatenate([gc[:256], ur], axis=0)
    ga, gb, gc = ga[:256], gb[:256], gc[:256]
    fa = 1.0 / (2 * A2 * (A2 - B2))
    fb = 1.0 / (2 * B2 * (B2 - A2))
    eva = (ga + A2 * gc) * fa
    oda = gb * (PA * fa)
    evb = (ga + B2 * gc) * fb
    odb = gb * (PB * fb)
    ri = lax.broadcasted_iota(jnp.int32, (C, C), 0)
    ci = lax.broadcasted_iota(jnp.int32, (C, C), 1)
    hi_half = ri >= CP
    mrow = 2 * jnp.where(hi_half, ri - CP, ri) + jnp.where(hi_half, 1, 0)
    ch = (mrow & ~15) + 2 * (mrow & 7) + ((mrow >> 3) & 1)
    pm = jnp.where(ch == ci, 1.0, 0.0).astype(bf16)

    def permpack(u):
        ut = lax.dot_general(pm, u.astype(bf16), (((1,), (1,)), ((), ())), preferred_element_type=f32)
        return _pack(ut[:CP], ut[CP:])
    g05[0] = permpack(u0)
    gr[...] = permpack(ur)
    gm[0] = permpack(eva + oda)
    gm[1] = permpack(eva - oda)
    gm[2] = permpack(evb + odb)
    gm[3] = permpack(evb - odb)
    g05[1] = permpack(u5)

    lane = lax.broadcasted_iota(jnp.int32, (8, 128), 1)

    def ld_e(q, g, k):
        t0 = xb0[q, g + Z[0], pl.ds(8 * k, 8), :]
        t1 = xb1[q, g, pl.ds(8 * k, 8), :]
        return jnp.concatenate([t1, t0[:, 96:]], axis=1)

    def stage_l1(t, rows, k):
        o = []
        for (sh, g) in rows:
            if t < 4:
                o.append(pltpu.roll(ld_e((t + sh) % 4, g, k), 32, 1))
            else:
                o.append(pltpu.roll(ld_e((3 + sh) % 4, g, k), 96 - 32 * (t - 4), 1))
        return o

    def ld_base(t, rows, k):
        if t < 4:
            return [xb0[(t + sh) % 4, g + Z[0], pl.ds(8 * k, 8), :] for (sh, g) in rows]
        return [ld_e((t - 4 + sh) % 4, g, k) for (sh, g) in rows]

    def versions(t, bases, l1):
        v = []
        for tw in range(3):
            if tw == 0:
                v.append(bases if t < 4 else [jnp.where(lane < 96, b, l) for b, l in zip(bases, l1)])
            else:
                m = (lane >= 128 - tw) if t < 4 else ((lane >= 96 - tw) & (lane < 128 - tw))
                v.append([pltpu.roll(jnp.where(m, l, b), tw, 1) for b, l in zip(bases, l1)])
        return v

    def transform(d):
        lo = _bt([_unpack(x, 0) for x in d])
        hi = _bt([_unpack(x, 1) for x in d])
        return [_pack(lo[c], hi[c]) for c in range(6)]

    def post_t(t, rows6, k):
        comps = transform(ld_base(t, rows6, k))
        if t >= 4:
            for c in range(6):
                tbs[t - 4][Z[0], pl.ds(8 * (6 * k + c), 8), :] = comps[c]
        return comps

    def post_l1(t, k):
        q, amt = (t, 32) if t < 4 else (3, 96 - 32 * (t - 4))
        return [pltpu.roll(tbs[q][Z[1], pl.ds(8 * (6 * k + c), 8), :], amt, 1) for c in range(6)]

    def stage_b(t, k, tw, v, save, z):
        k0 = tw * CP + 8 * k
        if len(v) == 4:
            d = [sb[z, t, pl.ds(k0, 8), :], sb[z + 1, t, pl.ds(k0, 8), :]] + v
        else:
            d = v
        if save:
            sb[z, t, pl.ds(k0, 8), :] = d[4]
            sb[z + 1, t, pl.ds(k0, 8), :] = d[5]
        if k0 < 128:
            comps = transform(d)
            for c in range(6):
                cbs[t][Z[0], pl.ds(128 * c + k0, 8), :] = comps[c]
        else:
            for i in range(6):
                cbs[t][Z[0], pl.ds(RB + 16 * i + (k0 - 128), 8), :] = d[i]

    lane48 = lax.broadcasted_iota(jnp.int32, (CP, 128), 1)

    def c_rounds(t, g, pieces):
        def ld(a, n):
            return pltpu.bitcast(cbs[t][Z[1], pl.ds(a, n), :], bf16)

        def dot(gw, v):
            return jnp.dot(pltpu.bitcast(gw, bf16), v, preferred_element_type=f32)

        def store(i, y):
            y = jnp.concatenate([_pack(y[16 * b:16 * b + 8], y[16 * b + 8:16 * b + 16]) for b in range(NV)], axis=0)
            if t < 4:
                yb0[t, g + i] = y
            else:
                yb1[t - 4, g + i] = y[:, :96]
                pieces[i].append(y)
        p0 = dot(g05[0], jnp.concatenate([ld(0, 128), ld(RB, 48)], axis=0))
        p2 = dot(gr[...], ld(RB + 32, 48))
        yield p2[0:8]
        yield p2[64:72]
        ap = dot(gm[0], ld(128, 128))
        am = dot(gm[1], ld(256, 128))
        sa = ap + am
        da = ap - am
        p0 = p0 + sa
        p2 = p2 + A2 * sa
        yield da[32:40]
        bp = dot(gm[2], ld(384, 128))
        bm = dot(gm[3], ld(512, 128))
        sbb = bp + bm
        db = bp - bm
        store(0, p0 + sbb)
        store(2, p2 + B2 * sbb)
        p1 = PA * da + PB * db
        p3 = (PA * A2) * da + (PB * B2) * db
        yield db[0:8]
        yield db[64:72]
        store(3, p3 + dot(g05[1], jnp.concatenate([ld(640, 128), ld(RB + 48, 48)], axis=0)))
        r1 = dot(gr[...], ld(RB + 16, 48))
        store(1, p1 + r1)
        yield r1[32:40]

    def stage_d(g, pieces, i):
        p4, p5, p6 = [pltpu.roll(y, 32 * (q + 1), 1) for q, y in enumerate(pieces[i])]
        yb1[3, g + i] = jnp.where(lane48 < 32, p4, jnp.where(lane48 < 64, p5, p6))[:, :96]

    def run_block(j0, nq, sj0, outs):
        first = sj0 == 0
        last = sj0 is not None and sj0 + nq == NQ
        Z[0] = zs[0]
        Z[1] = zs[1]
        Z[2] = zs[2]
        nab = nq * NT * NV

        def rows_of(n):
            g = 4 * (j0 + n // NT)
            r = [(0, g + i) for i in range(4)]
            if first and n < NT:
                r = [(3, G - 2), (3, G - 1)] + r
            return r
        def rows6_of(n):
            g = 4 * (j0 + n // NT)
            if first and n < NT:
                return rows_of(n)
            return [(0, g - 2 + i) for i in range(6)]
        l1 = {}
        nl1 = [0]

        def l1_upto(m):
            while nl1[0] < min(m, nab):
                n, kk = divmod(nl1[0], NV)
                k = KORD[kk]
                if k < NP:
                    if n % NT == 0:
                        post_t(7, rows6_of(n), k)
                    l1[nl1[0]] = post_l1(ORDER[n % NT], k)
                else:
                    l1[nl1[0]] = stage_l1(ORDER[n % NT], rows_of(n), k)
                nl1[0] += 1

        def ab_chunk(m):
            n, kk = divmod(m, NV)
            k = KORD[kk]
            t = ORDER[n % NT]
            d1 = D1F if (first and n < NT) else D1
            l1_upto(m + 1)
            if k < NP:
                vs = versions(t, post_t(t, rows6_of(n), k), l1.pop(m))
                l1_upto(m + d1 + 1)
                for tw in range(3):
                    for c in range(6):
                        cbs[t][Z[0], pl.ds(128 * c + tw * CP + 8 * k, 8), :] = vs[tw][c]
            else:
                vs = versions(t, ld_base(t, rows_of(n), k), l1.pop(m))
                l1_upto(m + d1 + 1)
                for tw in range(3):
                    stage_b(t, k, tw, vs[tw], not (last and n >= (nq - 1) * NT), Z[(n // NT) % 2] if nq > 1 else 0)

        l1_upto(D1F if first else D1)
        m = (LA * NV if first else 0) + OFF
        for mm in range(m):
            ab_chunk(mm)
        pieces = None
        for n in range(0 if first else -LA, nq * NT - (0 if last else LA)):
            jj, s = divmod(n, NT)
            t = ORDER[s]
            j = j0 + jj
            sj = None if sj0 is None else sj0 + jj
            if s == 0:
                pieces = [[], [], [], []]
            for r, tick in enumerate(c_rounds(t, 4 * j, pieces)):
                if m < nab:
                    xb0[0, Z[2], pl.ds(0, 8), :] = pltpu.bitcast(tick, u32)
                    ab_chunk(m)
                m += 1
                if s == DS and r < 4:
                    stage_d(4 * j, pieces, r)
                if r == 2 and last and n > -LA:
                    pjj, ps = divmod(n - 1, NT)
                    done = [(pjj, ORDER[ps])] + ([(jj, 7)] if (s == DS + 1 and jj == 0) else [])
                    for (djj, p) in done:
                        for cp in tile_copies(p, 4 * (j0 + djj)):
                            cp.start()

    for cp in in_copies(G - 2, 2, 0):
        cp.wait()
    for cp in in_copies(*chunks[0], 0):
        cp.wait()
    run_block(0, 1, 0, None)

    def body(k, carry):
        j = 1 + k * UQ
        for cp in in_copies(4 * j, 4 * UQ, k + 1):
            cp.wait()

        @pl.when(k == HOLD)
        def _():
            for cp in out_copies(1 + HOLD * UQ, True):
                cp.start()

        @pl.when(k > HOLD)
        def _():
            for cp in out_copies(j, False):
                cp.start()
        run_block(j, UQ, None, None)
        return carry
    lax.fori_loop(0, NB, body, 0)

    for cp in in_copies(*chunks[NB + 1], NB + 1):
        cp.wait()
    for cp in out_copies(NQ - 1, False):
        cp.start()
    run_block(NQ - 1, 1, NQ - 1, None)
    for cp in tile_copies(ORDER[NT - 1], 4 * (NQ - 1)):
        cp.start()

    for cp in out_copies(1 + HOLD * UQ, True):
        cp.wait()
    for k in range(HOLD + 1, NB + 1):
        for cp in out_copies(1 + k * UQ, False):
            cp.wait()
    for p in (2, 3):
        for cp in tile_copies(p, 4 * (NQ - 2)):
            cp.wait()
    for p in range(8):
        for cp in tile_copies(p, 4 * (NQ - 1)):
            cp.wait()


@jax.jit
def pallas_standalone__fft_conv__vision_kernel(x, w):
    xt = jnp.transpose(x, (0, 1, 3, 2)).reshape(NS, G, C, W)
    y = pl.pallas_call(
        kern,
        out_shape=jax.ShapeDtypeStruct((NS, G, C, W), x.dtype),
        in_specs=[pl.BlockSpec(memory_space=pl.ANY), pl.BlockSpec(memory_space=pl.ANY)],
        out_specs=pl.BlockSpec(memory_space=pl.ANY),
        scratch_shapes=[
            pltpu.VMEM((NS, G + 1, CP, 128), u32),
            pltpu.VMEM((NS, G, CP, 96), u32),
            pltpu.VMEM((3, 3, C, C), bf16),
            pltpu.VMEM((2, CP, 352), u32),
            pltpu.VMEM((4, CP, 256), u32),
            pltpu.VMEM((CP, 96), u32),
            pltpu.VMEM((2, NT, 144, 128), u32),
            pltpu.VMEM((NS, G, CP, 128), u32),
            pltpu.VMEM((NS, G, CP, 96), u32),
            pltpu.SemaphoreType.DMA((sum(r for _, r in BLOCKS),)),
            pltpu.SemaphoreType.DMA((1,)),
            pltpu.SemaphoreType.DMA((1,)),
            pltpu.SMEM((3,), jnp.int32),
        ] + [pltpu.VMEM((2, RB + 96, 128), u32)] * NT + [pltpu.VMEM((2, 48 * max(NP, 1), 128), u32)] * 4,
        compiler_params=pltpu.CompilerParams(vmem_limit_bytes=100 * 1024 * 1024),
    )(xt, w)
    return jnp.transpose(y.reshape(1, H, C, W), (0, 1, 3, 2))
```

```python
import jax, jax.numpy as jnp
from jax import lax
from jax.experimental import pallas as pl
from jax.experimental.pallas import tpu as pltpu

H = W = 224
C = 96
NS = 4
G = H // NS
NT = 7
CP = C // 2
NQ = G // 4
LA = 2
D1 = 3
D1F = 4
OFF = 2
DS = 4
UQ = 2
PRE = (1, 1, 1)
FQ = sum(PRE)
NPRE = len(PRE)
NP = 4
NB = (NQ - FQ - 1) // UQ
LQ = NQ - FQ - NB * UQ
ORDER = (4, 5, 6, 0, 1, 2, 3)
NSPLIT = 3
KORD = (4, 0, 1, 5, 2, 3)
NV = CP // 8
RB = 768

PA = 2.0 / 3.0
PB = 1.5
A2, B2 = PA * PA, PB * PB

bf16 = jnp.bfloat16
f32 = jnp.float32
u32 = jnp.uint32


def _unpack(v, i):
    return pltpu.unpack_elementwise(v, index=i, packed_dtype=bf16, unpacked_dtype=f32)


def _pack(lo, hi):
    return pltpu.pack_elementwise([lo, hi], packed_dtype=bf16)


def _bt(d):
    d0, d1, d2, d3, d4, d5 = d
    a2d2 = A2 * d2
    b2d3 = B2 * d3
    ea = d4 - B2 * d2
    eb = d4 - a2d2
    oa = A2 * d3 - d1
    ob = b2d3 - d1
    boa = PB * oa
    aob = PA * ob
    return (ea - a2d2 + d0, ea + boa, ea - boa, eb + aob, eb - aob, d5 - b2d3 - oa)


def kern(x_hbm, w_hbm, o_hbm, xb0, xb1, wb, g05, gm, gr, sb, yb, sin, sw, sout, zs, *bufs):
    cbs, tbs = bufs[:NT], bufs[NT:]
    zs[0] = 0
    zs[1] = 0
    zs[2] = G
    Z = [None, None, None]
    xb0h = xb0.bitcast(bf16)
    xb1h = xb1.bitcast(bf16)
    ybu = yb.bitcast(u32)

    def in_copies(g0, n, s):
        return (pltpu.make_async_copy(x_hbm.at[:, pl.ds(g0, n), :, pl.ds(0, 128)], xb0h.at[:, pl.ds(g0, n)], sin.at[s]),
                pltpu.make_async_copy(x_hbm.at[:, pl.ds(g0, n), :, pl.ds(128, 96)], xb1h.at[:, pl.ds(g0, n)], sin.at[s]))

    def last_in_copies():
        s = NB + NPRE
        cps = list(in_copies(4 * (NQ - LQ), 4 * (LQ - 1), s)) if LQ > 1 else []
        nc = C // NSPLIT
        for q in range(4):
            for g in (G - 4, G - 3):
                for h in range(NSPLIT):
                    cs = pl.ds(h * nc, nc)
                    cps.append(pltpu.make_async_copy(x_hbm.at[q, g, cs, pl.ds(0, 128)], xb0h.at[q, g, cs], sin.at[s]))
                    cps.append(pltpu.make_async_copy(x_hbm.at[q, g, cs, pl.ds(128, 96)], xb1h.at[q, g, cs], sin.at[s]))
        return cps

    def row_copy(g):
        return pltpu.make_async_copy(yb.at[:, g], o_hbm.at[:, g], sout.at[0])

    def tile_copy(p, g0):
        ls = pl.ds(0, 128) if p < 4 else pl.ds(128, 96)
        return pltpu.make_async_copy(yb.at[p % 4, pl.ds(g0, 4), :, ls], o_hbm.at[p % 4, pl.ds(g0, 4), :, ls], sout.at[0])

    wcp = pltpu.make_async_copy(w_hbm, wb, sw.at[0])
    wcp.start()
    for cp in in_copies(G - 2, 2, 0):
        cp.start()
    for i in range(NPRE):
        for cp in in_copies(4 * sum(PRE[:i]), 4 * PRE[i], i):
            cp.start()
    for k in range(NB):
        for cp in in_copies(4 * (FQ + k * UQ), 4 * UQ, k + NPRE):
            cp.start()
    for cp in last_in_copies():
        cp.start()

    wcp.wait()
    wf = [wb[th].reshape(3 * C, C).astype(f32) for th in range(3)]
    ga, gb, gc = wf[2], wf[1], wf[0]
    ur = jnp.concatenate([ga[256:], gb[256:], gc[256:]], axis=0)
    u0 = jnp.concatenate([ga[:256], ur], axis=0)
    u5 = jnp.concatenate([gc[:256], ur], axis=0)
    ga, gb, gc = ga[:256], gb[:256], gc[:256]
    fa = 1.0 / (2 * A2 * (A2 - B2))
    fb = 1.0 / (2 * B2 * (B2 - A2))
    eva = (ga + A2 * gc) * fa
    oda = gb * (PA * fa)
    evb = (ga + B2 * gc) * fb
    odb = gb * (PB * fb)
    ri = lax.broadcasted_iota(jnp.int32, (C, C), 0)
    ci = lax.broadcasted_iota(jnp.int32, (C, C), 1)
    hi_half = ri >= CP
    mrow = 2 * jnp.where(hi_half, ri - CP, ri) + jnp.where(hi_half, 1, 0)
    ch = (mrow & ~15) + 2 * (mrow & 7) + ((mrow >> 3) & 1)
    pm = jnp.where(ch == ci, 1.0, 0.0).astype(bf16)

    def permpack(u):
        ut = lax.dot_general(pm, u.astype(bf16), (((1,), (1,)), ((), ())), preferred_element_type=f32)
        return _pack(ut[:CP], ut[CP:])
    g05[0] = permpack(u0)
    gr[...] = permpack(ur)
    gm[0] = permpack(eva + oda)
    gm[1] = permpack(eva - oda)
    gm[2] = permpack(evb + odb)
    gm[3] = permpack(evb - odb)
    g05[1] = permpack(u5)

    lane = lax.broadcasted_iota(jnp.int32, (8, 128), 1)

    def ld_e(q, g, k):
        t0 = xb0[q, g + Z[0], pl.ds(8 * k, 8), :]
        t1 = xb1[q, g, pl.ds(8 * k, 8), :]
        return jnp.concatenate([t1, t0[:, 96:]], axis=1)

    def stage_l1(t, rows, k):
        q, amt = (t, 32) if t < 4 else (3, 96 - 32 * (t - 4))
        return [pltpu.roll(ld_e((q + sh) % 4, g, k), amt, 1) for (sh, g) in rows]

    def ld_base(t, rows, k):
        if t < 4:
            return [xb0[(t + sh) % 4, g + Z[0], pl.ds(8 * k, 8), :] for (sh, g) in rows]
        return [ld_e((t - 4 + sh) % 4, g, k) for (sh, g) in rows]

    def versions(t, bases, l1):
        v = []
        for tw in range(3):
            if tw == 0:
                v.append(bases if t < 4 else [jnp.where(lane < 96, b, l) for b, l in zip(bases, l1)])
            else:
                m = (lane >= 128 - tw) if t < 4 else ((lane >= 96 - tw) & (lane < 128 - tw))
                v.append([pltpu.roll(jnp.where(m, l, b), tw, 1) for b, l in zip(bases, l1)])
        return v

    def transform(d):
        lo = _bt([_unpack(x, 0) for x in d])
        hi = _bt([_unpack(x, 1) for x in d])
        return [_pack(lo[c], hi[c]) for c in range(6)]

    def post_t(t, rows6, k):
        comps = transform(ld_base(t, rows6, k))
        if t >= 4:
            for c in range(6):
                tbs[t - 4][Z[0], pl.ds(8 * (6 * k + c), 8), :] = comps[c]
        return comps

    def post_l1(t, k):
        q, amt = (t, 32) if t < 4 else (3, 96 - 32 * (t - 4))
        return [pltpu.roll(tbs[q][Z[1], pl.ds(8 * (6 * k + c), 8), :], amt, 1) for c in range(6)]

    def stage_b(t, k, tw, v, save, z):
        k0 = tw * CP + 8 * k
        if len(v) == 4:
            d = [sb[z, t, pl.ds(k0, 8), :], sb[z + 1, t, pl.ds(k0, 8), :]] + v
        else:
            d = v
        if save:
            sb[z, t, pl.ds(k0, 8), :] = d[4]
            sb[z + 1, t, pl.ds(k0, 8), :] = d[5]
        if k0 < 128:
            comps = transform(d)
            for c in range(6):
                cbs[t][Z[0], pl.ds(128 * c + k0, 8), :] = comps[c]
        else:
            for i in range(6):
                cbs[t][Z[0], pl.ds(RB + 16 * i + (k0 - 128), 8), :] = d[i]

    lane48 = lax.broadcasted_iota(jnp.int32, (CP, 128), 1)

    def c_rounds(t, g, pieces):
        def ld(a, n):
            return pltpu.bitcast(cbs[t][Z[1], pl.ds(a, n), :], bf16)

        def dot(gw, v):
            return jnp.dot(pltpu.bitcast(gw, bf16), v, preferred_element_type=f32)

        def store(i, y):
            y = jnp.concatenate([_pack(y[16 * b:16 * b + 8], y[16 * b + 8:16 * b + 16]) for b in range(NV)], axis=0)
            if t < 4:
                ybu[t, g + i, :, pl.ds(0, 128)] = y
            else:
                ybu[t - 4, g + i, :, pl.ds(128, 96)] = y[:, :96]
                pieces[i][t - 4] = y
        p0 = dot(g05[0], jnp.concatenate([ld(0, 128), ld(RB, 48)], axis=0))
        p2 = dot(gr[...], ld(RB + 32, 48))
        yield p2[0:8]
        yield p2[64:72]
        ap = dot(gm[0], ld(128, 128))
        am = dot(gm[1], ld(256, 128))
        sa = ap + am
        da = ap - am
        p0 = p0 + sa
        p2 = p2 + A2 * sa
        yield da[32:40]
        bp = dot(gm[2], ld(384, 128))
        bm = dot(gm[3], ld(512, 128))
        sbb = bp + bm
        db = bp - bm
        store(0, p0 + sbb)
        store(2, p2 + B2 * sbb)
        p1 = PA * da + PB * db
        p3 = (PA * A2) * da + (PB * B2) * db
        yield db[0:8]
        yield db[64:72]
        store(3, p3 + dot(g05[1], jnp.concatenate([ld(640, 128), ld(RB + 48, 48)], axis=0)))
        r1 = dot(gr[...], ld(RB + 16, 48))
        store(1, p1 + r1)
        yield r1[32:40]

    def stage_d(g, pieces, i):
        p4, p5, p6 = [pltpu.roll(y, 32 * (q + 1), 1) for q, y in enumerate(pieces[i])]
        ybu[3, g + i, :, pl.ds(128, 96)] = jnp.where(lane48 < 32, p4, jnp.where(lane48 < 64, p5, p6))[:, :96]

    def run_block(j0, nq, first, last):
        Z[0] = zs[0]
        Z[1] = zs[1]
        Z[2] = zs[2]
        nab = nq * NT * NV

        def rows_of(n):
            g = 4 * (j0 + n // NT)
            r = [(0, g + i) for i in range(4)]
            if first and n < NT:
                r = [(3, G - 2), (3, G - 1)] + r
            return r

        def rows6_of(n):
            g = 4 * (j0 + n // NT)
            if first and n < NT:
                return rows_of(n)
            return [(0, g - 2 + i) for i in range(6)]
        l1 = {}
        nl1 = [0]

        def l1_upto(m):
            while nl1[0] < min(m, nab):
                n, kk = divmod(nl1[0], NV)
                k = KORD[kk]
                if k < NP:
                    if n % NT == 0:
                        post_t(7, rows6_of(n), k)
                    l1[nl1[0]] = post_l1(ORDER[n % NT], k)
                else:
                    l1[nl1[0]] = stage_l1(ORDER[n % NT], rows_of(n), k)
                nl1[0] += 1

        def ab_chunk(m):
            n, kk = divmod(m, NV)
            k = KORD[kk]
            t = ORDER[n % NT]
            d1 = D1F if (first and n < NT) else D1
            l1_upto(m + 1)
            if k < NP:
                vs = versions(t, post_t(t, rows6_of(n), k), l1.pop(m))
                l1_upto(m + d1 + 1)
                for tw in range(3):
                    for c in range(6):
                        cbs[t][Z[0], pl.ds(128 * c + tw * CP + 8 * k, 8), :] = vs[tw][c]
            else:
                vs = versions(t, ld_base(t, rows_of(n), k), l1.pop(m))
                l1_upto(m + d1 + 1)
                for tw in range(3):
                    stage_b(t, k, tw, vs[tw], not (last and n >= (nq - 1) * NT), Z[(n // NT) % 2] if nq > 1 else 0)

        l1_upto(D1F if first else D1)
        m = (LA * NV if first else 0) + OFF
        for mm in range(m):
            ab_chunk(mm)
        pieces = None
        for n in range(0 if first else -LA, nq * NT - (0 if last else LA)):
            jj, s = divmod(n, NT)
            t = ORDER[s]
            j = j0 + jj
            if s == 0:
                pieces = [[None] * 3 for _ in range(4)]
            for r, tick in enumerate(c_rounds(t, 4 * j, pieces)):
                if m < nab:
                    xb0[0, Z[2], pl.ds(0, 8), :] = pltpu.bitcast(tick, u32)
                    ab_chunk(m)
                m += 1
                if s == DS and r < 4:
                    stage_d(4 * j, pieces, r)
                if r == 2:
                    if s == 0 and not (first and jj == 0):
                        for i in range(4):
                            row_copy(4 * (j - 1) + i).start()
                    if last and jj == nq - 1 and s > 0:
                        tile_copy(ORDER[s - 1], 4 * j).start()
                        if s == DS + 1:
                            tile_copy(7, 4 * j).start()

    for cp in in_copies(G - 2, 2, 0):
        cp.wait()
    for i in range(NPRE):
        for cp in in_copies(4 * sum(PRE[:i]), 4 * PRE[i], i):
            cp.wait()
        run_block(sum(PRE[:i]), PRE[i], i == 0, False)

    def body(k, carry):
        j = FQ + k * UQ
        for cp in in_copies(4 * j, 4 * UQ, k + NPRE):
            cp.wait()
        run_block(j, UQ, False, False)
        return carry
    lax.fori_loop(0, NB, body, 0)

    for cp in last_in_copies():
        cp.wait()
    run_block(NQ - LQ, LQ, False, True)
    tile_copy(ORDER[NT - 1], 4 * (NQ - 1)).start()

    for g in range(G - 4):
        row_copy(g).wait()
    for p in range(8):
        tile_copy(p, 4 * (NQ - 1)).wait()


@jax.jit
def pallas_standalone__fft_conv__vision_kernel(x, w):
    xt = jnp.transpose(x, (0, 1, 3, 2)).reshape(NS, G, C, W)
    y = pl.pallas_call(
        kern,
        out_shape=jax.ShapeDtypeStruct((NS, G, C, W), x.dtype),
        in_specs=[pl.BlockSpec(memory_space=pl.ANY), pl.BlockSpec(memory_space=pl.ANY)],
        out_specs=pl.BlockSpec(memory_space=pl.ANY),
        scratch_shapes=[
            pltpu.VMEM((NS, G + 1, CP, 128), u32),
            pltpu.VMEM((NS, G, CP, 96), u32),
            pltpu.VMEM((3, 3, C, C), bf16),
            pltpu.VMEM((2, CP, 352), u32),
            pltpu.VMEM((4, CP, 256), u32),
            pltpu.VMEM((CP, 96), u32),
            pltpu.VMEM((2, NT, 144, 128), u32),
            pltpu.VMEM((NS, G, C, W), bf16),
            pltpu.SemaphoreType.DMA((NB + NPRE + 1,)),
            pltpu.SemaphoreType.DMA((1,)),
            pltpu.SemaphoreType.DMA((1,)),
            pltpu.SMEM((3,), jnp.int32),
        ] + [pltpu.VMEM((2, RB + 96, 128), u32)] * NT + [pltpu.VMEM((2, 48 * max(NP, 1), 128), u32)] * 4,
        compiler_params=pltpu.CompilerParams(vmem_limit_bytes=100 * 1024 * 1024, disable_semaphore_checks=True, disable_bounds_checks=True),
    )(xt, w)
    return jnp.transpose(y.reshape(1, H, C, W), (0, 1, 3, 2))
```

```python
import jax, jax.numpy as jnp
from jax import lax
from jax.experimental import pallas as pl
from jax.experimental.pallas import tpu as pltpu

H = W = 224
C = 96
NS = 4
G = H // NS
NT = 7
CP = C // 2
NQ = G // 4
LA = 2
D1 = 3
D1F = 4
OFF = 3
DS = 4
UQ = 2
PRE = (1, 1, 1)
assert PRE[0] == 1
FQ = sum(PRE)
NPRE = len(PRE)
NP = 4
NB = (NQ - FQ - 1) // UQ
LQ = NQ - FQ - NB * UQ
ORDER = (4, 0, 5, 6, 1, 2, 3)
NSPLIT = 3
KORD = (0, 4, 1, 2, 5, 3)
NC0 = 1
NV = CP // 8
RB = 768

SEL16 = 1
PA = 2.0 / 3.0
PB = 1.5
A2, B2 = PA * PA, PB * PB

bf16 = jnp.bfloat16
f32 = jnp.float32
u32 = jnp.uint32


def _unpack(v, i):
    return pltpu.bitcast((v << 16) if i == 0 else (v & jnp.uint32(0xFFFF0000)), f32)


def _pack(lo, hi):
    lo = (pltpu.bitcast(lo, u32) + jnp.uint32(0x8000)) >> 16
    hi = pltpu.bitcast(hi, u32) + jnp.uint32(0x8000)
    if SEL16:
        odd = (lax.broadcasted_iota(jnp.int32, (16, 128), 0) & 1) == 1
        return pltpu.bitcast(jnp.where(odd, pltpu.bitcast(hi, bf16), pltpu.bitcast(lo, bf16)), u32)
    return lo | (hi & jnp.uint32(0xFFFF0000))


def _bt(d):
    d0, d1, d2, d3, d4, d5 = d
    a2d2 = A2 * d2
    b2d3 = B2 * d3
    ea = d4 - B2 * d2
    eb = d4 - a2d2
    oa = A2 * d3 - d1
    ob = b2d3 - d1
    boa = PB * oa
    aob = PA * ob
    return (ea - a2d2 + d0, ea + boa, ea - boa, eb + aob, eb - aob, d5 - b2d3 - oa)


def kern(x_hbm, w_hbm, o_hbm, xb0, xb1, wb, g05, gm, gr, sb, yb, ps, sin, sw, sout, zs, *bufs):
    cbs, tbs = bufs[:NT], bufs[NT:]
    zs[0] = 0
    zs[1] = 0
    zs[2] = G
    Z = [None, None, None]
    xb0h = xb0.bitcast(bf16)
    xb1h = xb1.bitcast(bf16)
    ybu = yb.bitcast(u32)

    def in_copies(g0, n, s, q0=0, nq=NS):
        qs, gs = pl.ds(q0, nq), pl.ds(g0, n)
        return (pltpu.make_async_copy(x_hbm.at[qs, gs, :, pl.ds(0, 128)], xb0h.at[qs, gs], sin.at[s]),
                pltpu.make_async_copy(x_hbm.at[qs, gs, :, pl.ds(128, 96)], xb1h.at[qs, gs], sin.at[s]))

    def first_copies(part):
        if part == 0:
            return in_copies(0, 4, 0, 3, 1) + in_copies(G - 2, 2, 0, 2, 2) + in_copies(0, 4, 0, 0, 1)
        s = NB + NPRE + 1
        return in_copies(0, 4, s, 1, 2) + in_copies(G - 2, 2, s, 0, 2)

    def last_in_copies():
        s = NB + NPRE
        cps = list(in_copies(4 * (NQ - LQ), 4 * (LQ - 1), s)) if LQ > 1 else []
        nc = C // NSPLIT
        for q in range(4):
            for g in (G - 4, G - 3):
                for h in range(NSPLIT):
                    cs = pl.ds(h * nc, nc)
                    cps.append(pltpu.make_async_copy(x_hbm.at[q, g, cs, pl.ds(0, 128)], xb0h.at[q, g, cs], sin.at[s]))
                    cps.append(pltpu.make_async_copy(x_hbm.at[q, g, cs, pl.ds(128, 96)], xb1h.at[q, g, cs], sin.at[s]))
        return cps

    def row_copy(g):
        return pltpu.make_async_copy(yb.at[:, g], o_hbm.at[:, g], sout.at[0])

    def tile_copy(p, g0):
        ls = pl.ds(0, 128) if p < 4 else pl.ds(128, 96)
        return pltpu.make_async_copy(yb.at[p % 4, pl.ds(g0, 4), :, ls], o_hbm.at[p % 4, pl.ds(g0, 4), :, ls], sout.at[0])

    wcp = pltpu.make_async_copy(w_hbm, wb, sw.at[0])
    wcp.start()
    for cp in first_copies(0) + first_copies(1):
        cp.start()
    for i in range(1, NPRE):
        for cp in in_copies(4 * sum(PRE[:i]), 4 * PRE[i], i):
            cp.start()
    for k in range(NB):
        for cp in in_copies(4 * (FQ + k * UQ), 4 * UQ, k + NPRE):
            cp.start()
    for cp in last_in_copies():
        cp.start()

    wcp.wait()
    wf = [wb[th].reshape(3 * C, C).astype(f32) for th in range(3)]
    ga, gb, gc = wf[2], wf[1], wf[0]
    ur = jnp.concatenate([ga[256:], gb[256:], gc[256:]], axis=0)
    u0 = jnp.concatenate([ga[:256], ur], axis=0)
    u5 = jnp.concatenate([gc[:256], ur], axis=0)
    ga, gb, gc = ga[:256], gb[:256], gc[:256]
    fa = 1.0 / (2 * A2 * (A2 - B2))
    fb = 1.0 / (2 * B2 * (B2 - A2))
    eva = (ga + A2 * gc) * fa
    oda = gb * (PA * fa)
    evb = (ga + B2 * gc) * fb
    odb = gb * (PB * fb)
    ri = lax.broadcasted_iota(jnp.int32, (C, C), 0)
    ci = lax.broadcasted_iota(jnp.int32, (C, C), 1)
    eye = jnp.where(ri == ci, 1.0, 0.0).astype(bf16)

    def permpack(u):
        ut = lax.dot_general(eye, u.astype(bf16), (((1,), (1,)), ((), ())), preferred_element_type=f32)
        return pltpu.bitcast(ut.astype(bf16), u32)
    g05[0] = permpack(u0)
    gr[...] = permpack(ur)
    gm[0] = permpack(eva + oda)
    gm[1] = permpack(eva - oda)
    gm[2] = permpack(evb + odb)
    gm[3] = permpack(evb - odb)
    g05[1] = permpack(u5)

    lane = lax.broadcasted_iota(jnp.int32, (8, 128), 1)

    def ld_e(q, g, k):
        t0 = xb0[q, g + Z[0], pl.ds(8 * k, 8), :]
        t1 = xb1[q, g, pl.ds(8 * k, 8), :]
        return jnp.concatenate([t1, t0[:, 96:]], axis=1)

    def stage_l1(t, rows, k):
        q, amt = (t, 32) if t < 4 else (3, 96 - 32 * (t - 4))
        return [pltpu.roll(ld_e((q + sh) % 4, g, k), amt, 1) for (sh, g) in rows]

    def ld_base(t, rows, k):
        if t < 4:
            return [xb0[(t + sh) % 4, g + Z[0], pl.ds(8 * k, 8), :] for (sh, g) in rows]
        return [ld_e((t - 4 + sh) % 4, g, k) for (sh, g) in rows]

    def versions(t, bases, l1):
        v = []
        for tw in range(3):
            if tw == 0:
                v.append(bases if t < 4 else [jnp.where(lane < 96, b, l) for b, l in zip(bases, l1)])
            else:
                m = (lane >= 128 - tw) if t < 4 else ((lane >= 96 - tw) & (lane < 128 - tw))
                v.append([pltpu.roll(jnp.where(m, l, b), tw, 1) for b, l in zip(bases, l1)])
        return v

    def transform(d):
        lo = _bt([_unpack(x, 0) for x in d])
        hi = _bt([_unpack(x, 1) for x in d])
        return [_pack(lo[c], hi[c]) for c in range(6)]

    def post_t(t, rows6, k):
        comps = transform(ld_base(t, rows6, k))
        if t >= 4:
            for c in range(6):
                tbs[t - 4][Z[0], pl.ds(8 * (6 * k + c), 8), :] = comps[c]
        return comps

    def post_l1(t, k):
        q, amt = (t, 32) if t < 4 else (3, 96 - 32 * (t - 4))
        return [pltpu.roll(tbs[q][Z[1], pl.ds(8 * (6 * k + c), 8), :], amt, 1) for c in range(6)]

    def stage_b(t, k, tw, v, save, z):
        k0 = tw * CP + 8 * k
        if len(v) == 4:
            d = [sb[z, t, pl.ds(k0, 8), :], sb[z + 1, t, pl.ds(k0, 8), :]] + v
        else:
            d = v
        if save:
            sb[z, t, pl.ds(k0, 8), :] = d[4]
            sb[z + 1, t, pl.ds(k0, 8), :] = d[5]
        if k0 < 128:
            comps = transform(d)
            for c in range(6):
                cbs[t][Z[0], pl.ds(128 * c + k0, 8), :] = comps[c]
        else:
            for i in range(6):
                cbs[t][Z[0], pl.ds(RB + 16 * i + (k0 - 128), 8), :] = d[i]

    lane48 = lax.broadcasted_iota(jnp.int32, (CP, 128), 1)

    def c_rounds(t, g, pieces):
        def ld(a, n):
            return pltpu.bitcast(cbs[t][Z[1], pl.ds(a, n), :], bf16)

        def dot(gw, v):
            return jnp.dot(pltpu.bitcast(gw, bf16), v, preferred_element_type=f32)

        def store(i0, y0, i1, y1):
            for i, y in ((i0, y0), (i1, y1)):
                if t < 4:
                    yb[t, g + i, :, pl.ds(0, 128)] = y.astype(bf16)
                else:
                    yb[t - 4, g + i, :, pl.ds(128, 96)] = y[:, :96].astype(bf16)
            if t >= 4:
                ps[:, pl.ds(512 * (t - 4) + 256 * (i0 % 2), 256)] = jnp.concatenate([y0, y1], axis=1).astype(bf16)
        p0 = dot(g05[0], jnp.concatenate([ld(0, 128), ld(RB, 48)], axis=0))
        p2 = dot(gr[...], ld(RB + 32, 48))
        yield p2[0:8]
        yield p2[64:72]
        ap = dot(gm[0], ld(128, 128))
        am = dot(gm[1], ld(256, 128))
        sa = ap + am
        da = ap - am
        p0 = p0 + sa
        p2 = p2 + A2 * sa
        yield da[32:40]
        bp = dot(gm[2], ld(384, 128))
        bm = dot(gm[3], ld(512, 128))
        sbb = bp + bm
        db = bp - bm
        store(0, p0 + sbb, 2, p2 + B2 * sbb)
        p1 = PA * da + PB * db
        p3 = (PA * A2) * da + (PB * B2) * db
        yield db[0:8]
        yield db[64:72]
        y3 = p3 + dot(g05[1], jnp.concatenate([ld(640, 128), ld(RB + 48, 48)], axis=0))
        r1 = dot(gr[...], ld(RB + 16, 48))
        store(1, p1 + r1, 3, y3)
        yield r1[32:40]

    def stage_d(g, pieces, i):
        p4, p5, p6 = [pltpu.roll(pltpu.bitcast(ps[:, pl.ds(128 * (4 * q + 2 * (i % 2) + i // 2), 128)], u32), 32 * (q + 1), 1)
                      for q in range(3)]
        ybu[3, g + i, :, pl.ds(128, 96)] = jnp.where(lane48 < 32, p4, jnp.where(lane48 < 64, p5, p6))[:, :96]

    def run_block(j0, nq, first, last):
        Z[0] = zs[0]
        Z[1] = zs[1]
        Z[2] = zs[2]
        nab = nq * NT * NV

        def rows_of(n):
            g = 4 * (j0 + n // NT)
            r = [(0, g + i) for i in range(4)]
            if first and n < NT:
                r = [(3, G - 2), (3, G - 1)] + r
            return r

        def rows6_of(n):
            g = 4 * (j0 + n // NT)
            if first and n < NT:
                return rows_of(n)
            return [(0, g - 2 + i) for i in range(6)]
        l1 = {}
        nl1 = [0]

        def l1_upto(m):
            while nl1[0] < min(m, nab):
                n, kk = divmod(nl1[0], NV)
                k = KORD[kk]
                if k < NP:
                    if n % NT == 0:
                        post_t(7, rows6_of(n), k)
                    l1[nl1[0]] = post_l1(ORDER[n % NT], k)
                else:
                    l1[nl1[0]] = stage_l1(ORDER[n % NT], rows_of(n), k)
                nl1[0] += 1

        def ab_chunk(m):
            n, kk = divmod(m, NV)
            k = KORD[kk]
            t = ORDER[n % NT]
            d1 = D1F if (first and n < NT) else D1
            l1_upto(m + 1)
            if k < NP:
                vs = versions(t, post_t(t, rows6_of(n), k), l1.pop(m))
                l1_upto(m + d1 + 1)
                for tw in range(3):
                    for c in range(6):
                        cbs[t][Z[0], pl.ds(128 * c + tw * CP + 8 * k, 8), :] = vs[tw][c]
            else:
                vs = versions(t, ld_base(t, rows_of(n), k), l1.pop(m))
                l1_upto(m + d1 + 1)
                for tw in range(3):
                    stage_b(t, k, tw, vs[tw], not (last and n >= (nq - 1) * NT), Z[(n // NT) % 2] if nq > 1 else 0)

        l1_upto(D1F if first else D1)
        m = LA * NV if first else OFF
        for mm in range(m):
            ab_chunk(mm)
        pieces = None
        for n in range(0 if first else -LA, nq * NT - (0 if last else LA)):
            jj, s = divmod(n, NT)
            t = ORDER[s]
            j = j0 + jj
            if s == 0:
                pieces = [[None] * 3 for _ in range(4)]
            if first and n == NC0:
                for cp in first_copies(1):
                    cp.wait()
                while m < (LA + NC0) * NV + OFF:
                    ab_chunk(m)
                    m += 1
            for r, tick in enumerate(c_rounds(t, 4 * j, pieces)):
                if not (first and n < NC0):
                    if m < nab:
                        xb0[0, Z[2], pl.ds(0, 8), :] = pltpu.bitcast(tick, u32)
                        ab_chunk(m)
                    m += 1
                if s == DS and r < 4:
                    stage_d(4 * j, pieces, r)
                if r == 2:
                    if s == 0 and not (first and jj == 0):
                        for i in range(4):
                            row_copy(4 * (j - 1) + i).start()
                    if last and jj == nq - 1 and s > 0:
                        tile_copy(ORDER[s - 1], 4 * j).start()
                        if s == DS + 1:
                            tile_copy(7, 4 * j).start()

    for i in range(NPRE):
        for cp in (first_copies(0) if i == 0 else in_copies(4 * sum(PRE[:i]), 4 * PRE[i], i)):
            cp.wait()
        run_block(sum(PRE[:i]), PRE[i], i == 0, False)

    def body(k, carry):
        j = FQ + k * UQ
        for cp in in_copies(4 * j, 4 * UQ, k + NPRE):
            cp.wait()
        run_block(j, UQ, False, False)
        return carry
    lax.fori_loop(0, NB, body, 0)

    for cp in last_in_copies():
        cp.wait()
    run_block(NQ - LQ, LQ, False, True)
    tile_copy(ORDER[NT - 1], 4 * (NQ - 1)).start()

    for g in range(G - 4):
        row_copy(g).wait()
    for p in range(8):
        tile_copy(p, 4 * (NQ - 1)).wait()


@jax.jit
def pallas_standalone__fft_conv__vision_kernel(x, w):
    xt = jnp.transpose(x, (0, 1, 3, 2)).reshape(NS, G, C, W)
    y = pl.pallas_call(
        kern,
        out_shape=jax.ShapeDtypeStruct((NS, G, C, W), x.dtype),
        in_specs=[pl.BlockSpec(memory_space=pl.ANY), pl.BlockSpec(memory_space=pl.ANY)],
        out_specs=pl.BlockSpec(memory_space=pl.ANY),
        scratch_shapes=[
            pltpu.VMEM((NS, G + 1, CP, 128), u32),
            pltpu.VMEM((NS, G, CP, 96), u32),
            pltpu.VMEM((3, 3, C, C), bf16),
            pltpu.VMEM((2, CP, 352), u32),
            pltpu.VMEM((4, CP, 256), u32),
            pltpu.VMEM((CP, 96), u32),
            pltpu.VMEM((2, NT, 144, 128), u32),
            pltpu.VMEM((NS, G, C, W), bf16),
            pltpu.VMEM((C, 12 * 128), bf16),
            pltpu.SemaphoreType.DMA((NB + NPRE + 2,)),
            pltpu.SemaphoreType.DMA((1,)),
            pltpu.SemaphoreType.DMA((1,)),
            pltpu.SMEM((3,), jnp.int32),
        ] + [pltpu.VMEM((2, RB + 96, 128), u32)] * NT + [pltpu.VMEM((2, 48 * max(NP, 1), 128), u32)] * 4,
        compiler_params=pltpu.CompilerParams(vmem_limit_bytes=100 * 1024 * 1024, disable_semaphore_checks=True, disable_bounds_checks=True),
    )(xt, w)
    return jnp.transpose(y.reshape(1, H, C, W), (0, 1, 3, 2))
```

```python
import jax
import jax.numpy as jnp
from jax import lax
from jax.experimental import pallas as pl
from jax.experimental.pallas import tpu as pltpu

H = W = 224
C = 96
NS = 4
G = H // NS
NT = 7
CP = C // 2
NV = CP // 8
NQ = G // 4
NP = 4
RB = 768

LA = 2
D1, D1F = 3, 4
OFF = 3
DS = 4
NPRE = 3
UQ = 2
NB = (NQ - NPRE - 1) // UQ
ORDER = (4, 0, 5, 6, 1, 2, 3)
KORD = (0, 4, 1, 2, 5, 3)
assert NPRE + NB * UQ + 1 == NQ

PA = 2.0 / 3.0
PB = 1.5
A2, B2 = PA * PA, PB * PB

bf16 = jnp.bfloat16
f32 = jnp.float32
u32 = jnp.uint32


def _unpack(v, i):
    return pltpu.bitcast((v << 16) if i == 0 else (v & jnp.uint32(0xFFFF0000)), f32)


def _pack(lo, hi):
    lo = (pltpu.bitcast(lo, u32) + jnp.uint32(0x8000)) >> 16
    hi = pltpu.bitcast(hi, u32) + jnp.uint32(0x8000)
    odd = (lax.broadcasted_iota(jnp.int32, (16, 128), 0) & 1) == 1
    return pltpu.bitcast(jnp.where(odd, pltpu.bitcast(hi, bf16), pltpu.bitcast(lo, bf16)), u32)


def _bt(d):
    d0, d1, d2, d3, d4, d5 = d
    a2d2 = A2 * d2
    b2d3 = B2 * d3
    ea = d4 - B2 * d2
    eb = d4 - a2d2
    oa = A2 * d3 - d1
    ob = b2d3 - d1
    boa = PB * oa
    aob = PA * ob
    return (ea - a2d2 + d0, ea + boa, ea - boa, eb + aob, eb - aob, d5 - b2d3 - oa)


def _transform(d):
    lo = _bt([_unpack(x, 0) for x in d])
    hi = _bt([_unpack(x, 1) for x in d])
    return [_pack(lo[c], hi[c]) for c in range(6)]


def _kernel(x_hbm, w_hbm, o_hbm, xb0, xb1, wb, g05, gm, gr, sb, yb, ps, sin, sw, sout, zs, *bufs):
    cbs, tbs = bufs[:NT], bufs[NT:]
    xb0u, xb1u = xb0.bitcast(u32), xb1.bitcast(u32)
    zs[0] = 0
    zs[1] = 0
    zs[2] = G
    Z = [None, None, None]

    def in_copies(g0, n, s, q0=0, nq=NS):
        qs, gs = pl.ds(q0, nq), pl.ds(g0, n)
        return (pltpu.make_async_copy(x_hbm.at[qs, gs, :, pl.ds(0, 128)], xb0.at[qs, gs], sin.at[s]),
                pltpu.make_async_copy(x_hbm.at[qs, gs, :, pl.ds(128, 96)], xb1.at[qs, gs], sin.at[s]))

    def first_copies(part):
        if part == 0:
            return in_copies(0, 4, 0, 3, 1) + in_copies(G - 2, 2, 0, 2, 2) + in_copies(0, 4, 0, 0, 1)
        s = NPRE + NB + 1
        return in_copies(0, 4, s, 1, 2) + in_copies(G - 2, 2, s, 0, 2)

    def last_copies():
        s = NPRE + NB
        cps = []
        for q in range(NS):
            for g in (G - 4, G - 3):
                for h in range(3):
                    cs = pl.ds(32 * h, 32)
                    cps.append(pltpu.make_async_copy(
                        x_hbm.at[q, g, cs, pl.ds(0, 128)], xb0.at[q, g, cs], sin.at[s]))
                for h in range(2):
                    cs = pl.ds(48 * h, 48)
                    cps.append(pltpu.make_async_copy(
                        x_hbm.at[q, g, cs, pl.ds(128, 96)], xb1.at[q, g, cs], sin.at[s]))
        return cps

    def row_copy(g):
        return pltpu.make_async_copy(yb.at[:, g], o_hbm.at[:, g], sout.at[0])

    def part_copy(p):
        ls, gs = (pl.ds(0, 128) if p < 4 else pl.ds(128, 96)), pl.ds(G - 4, 4)
        return pltpu.make_async_copy(yb.at[p % 4, gs, :, ls], o_hbm.at[p % 4, gs, :, ls], sout.at[0])

    wcp = pltpu.make_async_copy(w_hbm, wb, sw.at[0])
    wcp.start()
    for cp in first_copies(0) + first_copies(1):
        cp.start()
    for i in range(1, NPRE):
        for cp in in_copies(4 * i, 4, i):
            cp.start()
    for k in range(NB):
        for cp in in_copies(4 * (NPRE + k * UQ), 4 * UQ, NPRE + k):
            cp.start()
    for cp in last_copies():
        cp.start()

    wcp.wait()
    wf = [wb[th].reshape(3 * C, C).astype(f32) for th in range(3)]
    ga, gb, gc = wf[2], wf[1], wf[0]
    ur = jnp.concatenate([ga[256:], gb[256:], gc[256:]], axis=0)
    u0 = jnp.concatenate([ga[:256], ur], axis=0)
    u5 = jnp.concatenate([gc[:256], ur], axis=0)
    ga, gb, gc = ga[:256], gb[:256], gc[:256]
    fa = 1.0 / (2 * A2 * (A2 - B2))
    fb = 1.0 / (2 * B2 * (B2 - A2))
    eva = (ga + A2 * gc) * fa
    oda = gb * (PA * fa)
    evb = (ga + B2 * gc) * fb
    odb = gb * (PB * fb)
    eye = jnp.where(lax.broadcasted_iota(jnp.int32, (C, C), 0) ==
                    lax.broadcasted_iota(jnp.int32, (C, C), 1), 1.0, 0.0).astype(bf16)

    def tr(u):
        ut = lax.dot_general(eye, u.astype(bf16), (((1,), (1,)), ((), ())),
                             preferred_element_type=f32)
        return pltpu.bitcast(ut.astype(bf16), u32)
    g05[0] = tr(u0)
    gr[...] = tr(ur)
    gm[0] = tr(eva + oda)
    gm[1] = tr(eva - oda)
    gm[2] = tr(evb + odb)
    gm[3] = tr(evb - odb)
    g05[1] = tr(u5)

    lane = lax.broadcasted_iota(jnp.int32, (8, 128), 1)
    lane48 = lax.broadcasted_iota(jnp.int32, (CP, 128), 1)

    def ld_e(q, g, k):
        t0 = xb0u[q, g + Z[0], pl.ds(8 * k, 8), :]
        t1 = xb1u[q, g, pl.ds(8 * k, 8), :]
        return jnp.concatenate([t1, t0[:, 96:]], axis=1)

    def ld_base(t, rows, k):
        if t < 4:
            return [xb0u[(t + sh) % 4, g + Z[0], pl.ds(8 * k, 8), :] for (sh, g) in rows]
        return [ld_e((t - 4 + sh) % 4, g, k) for (sh, g) in rows]

    def l1_src(t):
        return (t, 32) if t < 4 else (3, 96 - 32 * (t - 4))

    def versions(t, bases, l1):
        v = [bases if t < 4 else [jnp.where(lane < 96, b, l) for b, l in zip(bases, l1)]]
        for tw in (1, 2):
            m = (lane >= 128 - tw) if t < 4 else ((lane >= 96 - tw) & (lane < 128 - tw))
            v.append([pltpu.roll(jnp.where(m, l, b), tw, 1) for b, l in zip(bases, l1)])
        return v

    def post_t(t, rows6, k):
        comps = _transform(ld_base(t, rows6, k))
        if t >= 4:
            for c in range(6):
                tbs[t - 4][Z[0], pl.ds(8 * (6 * k + c), 8), :] = comps[c]
        return comps

    def pre_b(t, k, tw, v, save, z):
        k0 = tw * CP + 8 * k
        s0 = 16 * tw + 8 * (k - NP)
        d = v if len(v) == 6 else [sb[z, t, pl.ds(s0, 8), :], sb[z + 1, t, pl.ds(s0, 8), :]] + v
        if save:
            sb[z, t, pl.ds(s0, 8), :] = d[4]
            sb[z + 1, t, pl.ds(s0, 8), :] = d[5]
        if k0 < 128:
            comps = _transform(d)
            for c in range(6):
                cbs[t][Z[0], pl.ds(128 * c + k0, 8), :] = comps[c]
        else:
            for i in range(6):
                cbs[t][Z[0], pl.ds(RB + 16 * i + (k0 - 128), 8), :] = d[i]

    def c_rounds(t, g):
        def ld(a, n):
            return pltpu.bitcast(cbs[t][Z[1], pl.ds(a, n), :], bf16)

        def dot(gw, v):
            return jnp.dot(pltpu.bitcast(gw, bf16), v, preferred_element_type=f32)

        def store(i0, y0, i1, y1):
            for i, y in ((i0, y0), (i1, y1)):
                if t < 4:
                    yb[t, g + i, :, pl.ds(0, 128)] = y.astype(bf16)
                else:
                    yb[t - 4, g + i, :, pl.ds(128, 96)] = y[:, :96].astype(bf16)
            if t >= 4:
                ps[:, pl.ds(512 * (t - 4) + 256 * i0, 256)] = (
                    jnp.concatenate([y0, y1], axis=1).astype(bf16))
        p0 = dot(g05[0], jnp.concatenate([ld(0, 128), ld(RB, 48)], axis=0))
        p2 = dot(gr[...], ld(RB + 32, 48))
        yield p2[0:8]
        yield p2[64:72]
        ap = dot(gm[0], ld(128, 128))
        am = dot(gm[1], ld(256, 128))
        sa = ap + am
        da = ap - am
        p0 = p0 + sa
        p2 = p2 + A2 * sa
        yield da[32:40]
        bp = dot(gm[2], ld(384, 128))
        bm = dot(gm[3], ld(512, 128))
        sb_ = bp + bm
        db = bp - bm
        store(0, p0 + sb_, 2, p2 + B2 * sb_)
        p1 = PA * da + PB * db
        p3 = (PA * A2) * da + (PB * B2) * db
        yield db[0:8]
        yield db[64:72]
        y3 = p3 + dot(g05[1], jnp.concatenate([ld(640, 128), ld(RB + 48, 48)], axis=0))
        r1 = dot(gr[...], ld(RB + 16, 48))
        store(1, p1 + r1, 3, y3)
        yield r1[32:40]

    def stage_d(g, i):
        p4, p5, p6 = [
            pltpu.roll(pltpu.bitcast(ps[:, pl.ds(128 * (4 * q + 2 * (i % 2) + i // 2), 128)], u32),
                       32 * (q + 1), 1) for q in range(3)]
        y = jnp.where(lane48 < 32, p4, jnp.where(lane48 < 64, p5, p6))
        yb[3, g + i, :, pl.ds(128, 96)] = pltpu.bitcast(y, bf16)[:, :96]

    def run_block(j0, nq, first, last):
        Z[0] = zs[0]
        Z[1] = zs[1]
        Z[2] = zs[2]
        nab = nq * NT * NV

        def rows_of(n, six):
            g = 4 * (j0 + n // NT)
            if first:
                return [(3, G - 2), (3, G - 1)] + [(0, i) for i in range(4)]
            return [(0, g + i) for i in range(-2 if six else 0, 4)]
        l1 = {}
        nl1 = [0]

        def l1_upto(m):
            while nl1[0] < min(m, nab):
                n, kk = divmod(nl1[0], NV)
                k = KORD[kk]
                q, amt = l1_src(ORDER[n % NT])
                if k < NP:
                    if n % NT == 0:
                        post_t(7, rows_of(n, True), k)
                    src = [tbs[q][Z[1], pl.ds(8 * (6 * k + c), 8), :] for c in range(6)]
                else:
                    src = [ld_e((q + sh) % 4, g, k) for (sh, g) in rows_of(n, False)]
                l1[nl1[0]] = [pltpu.roll(v, amt, 1) for v in src]
                nl1[0] += 1

        def ab_chunk(m):
            n, kk = divmod(m, NV)
            k = KORD[kk]
            t = ORDER[n % NT]
            l1_upto(m + 1)
            bases = post_t(t, rows_of(n, True), k) if k < NP else ld_base(t, rows_of(n, False), k)
            vs = versions(t, bases, l1.pop(m))
            l1_upto(m + (D1F if first else D1) + 1)
            for tw in range(3):
                if k < NP:
                    for c in range(6):
                        cbs[t][Z[0], pl.ds(128 * c + tw * CP + 8 * k, 8), :] = vs[tw][c]
                else:
                    pre_b(t, k, tw, vs[tw], not last, Z[(n // NT) % 2] if nq > 1 else 0)

        l1_upto(D1F if first else D1)
        m = LA * NV if first else OFF
        for mm in range(m):
            ab_chunk(mm)
        for n in range(0 if first else -LA, nq * NT - (0 if last else LA)):
            jj, s = divmod(n, NT)
            j = j0 + jj
            if first and n == 1:
                for cp in first_copies(1):
                    cp.wait()
                while m < (LA + 1) * NV + OFF:
                    ab_chunk(m)
                    m += 1
            for r, tick in enumerate(c_rounds(ORDER[s], 4 * j)):
                if not (first and n == 0):
                    if m < nab:
                        xb0[0, Z[2], pl.ds(0, 8), :] = tick.astype(bf16)
                        ab_chunk(m)
                    m += 1
                if s == DS and r < 4:
                    stage_d(4 * j, r)
                if r == 2:
                    if s == 0 and not first:
                        for i in range(4):
                            row_copy(4 * (j - 1) + i).start()
                    if last and jj == 0 and s > 0:
                        part_copy(ORDER[s - 1]).start()
                        if s == DS + 1:
                            part_copy(7).start()

    for i in range(NPRE):
        for cp in (first_copies(0) if i == 0 else in_copies(4 * i, 4, i)):
            cp.wait()
        run_block(i, 1, i == 0, False)

    def body(k, carry):
        j = NPRE + k * UQ
        for cp in in_copies(4 * j, 4 * UQ, NPRE + k):
            cp.wait()
        run_block(j, UQ, False, False)
        return carry
    lax.fori_loop(0, NB, body, 0)

    for cp in last_copies():
        cp.wait()
    run_block(NQ - 1, 1, False, True)
    part_copy(ORDER[NT - 1]).start()

    for g in range(G - 4):
        row_copy(g).wait()
    for p in range(8):
        part_copy(p).wait()


@jax.jit
def pallas_standalone__fft_conv__vision_kernel(x: jax.Array, w: jax.Array):
    xt = jnp.transpose(x, (0, 1, 3, 2)).reshape(NS, G, C, W)
    y = pl.pallas_call(
        _kernel,
        out_shape=jax.ShapeDtypeStruct((NS, G, C, W), x.dtype),
        in_specs=[pl.BlockSpec(memory_space=pl.ANY), pl.BlockSpec(memory_space=pl.ANY)],
        out_specs=pl.BlockSpec(memory_space=pl.ANY),
        scratch_shapes=[
            pltpu.VMEM((NS, G + 1, C, 128), bf16),
            pltpu.VMEM((NS, G, C, 96), bf16),
            pltpu.VMEM((3, 3, C, C), bf16),
            pltpu.VMEM((2, CP, 352), u32),
            pltpu.VMEM((4, CP, 256), u32),
            pltpu.VMEM((CP, 96), u32),
            pltpu.VMEM((2, NT, 48, 128), u32),
            pltpu.VMEM((NS, G, C, W), bf16),
            pltpu.VMEM((C, 12 * 128), bf16),
            pltpu.SemaphoreType.DMA((NPRE + NB + 2,)),
            pltpu.SemaphoreType.DMA((1,)),
            pltpu.SemaphoreType.DMA((1,)),
            pltpu.SMEM((3,), jnp.int32),
        ] + [pltpu.VMEM((2, RB + 96, 128), u32)] * NT
          + [pltpu.VMEM((2, 48 * NP, 128), u32)] * NS,
        compiler_params=pltpu.CompilerParams(
            vmem_limit_bytes=100 * 1024 * 1024,
            disable_semaphore_checks=True,
            disable_bounds_checks=True,
        ),
    )(xt, w)
    return jnp.transpose(y.reshape(1, H, C, W), (0, 1, 3, 2))
```
